```python
import os as _os
_os.environ.setdefault("JAX_PLATFORMS", "cpu")
import jax
import jax.numpy as jnp

def _softmax(x, axis=-1):
    return jax.nn.softmax(x, axis=axis)
def _gelu(x):
    return jax.nn.gelu(x, approximate=True)
def _silu(x):
    return jax.nn.silu(x)
def _sigmoid(x):
    return jax.nn.sigmoid(x)
def _layernorm(x, axis=-1, eps=1e-5):
    m = jnp.mean(x, axis=axis, keepdims=True)
    v = jnp.var(x, axis=axis, keepdims=True)
    return (x - m) / jnp.sqrt(v + eps)
def _scatter_add(tgt, idx, src, axis=0):
    return tgt.at[idx].add(src)
def _segment_sum(src, seg, n):
    return jax.ops.segment_sum(src, seg, n)
class _Rng:
    def __init__(self, key):
        self._k = key
    def _next(self):
        self._k, sub = jax.random.split(self._k)
        return sub
    def normal(self, shape):
        return jax.random.normal(self._next(), shape, dtype=jnp.bfloat16)
    def randint(self, lo, hi, shape):
        return jax.random.randint(self._next(), shape, lo, hi, dtype=jnp.int32)
    def uniform(self, shape, lo=0.0, hi=1.0):
        return jax.random.uniform(self._next(), shape, jnp.bfloat16, lo, hi)
    def permutation(self, n):
        return jax.random.permutation(self._next(), n)


kernel_name = 'interleave_layers__gqa_block_cached__dense_activation_mish__decode'

def setup_inputs():
    _rng = _Rng(jax.random.key(int.from_bytes(__import__("os").urandom(4), "little")))
    _w = (lambda a: (lambda t: t.astype(jnp.bfloat16) if jnp.issubdtype(t.dtype, jnp.floating) else t)(jnp.asarray(a)))
    def _A_setup():
        B, Sq, D = 1, 1, 512
        Hq, Hkv, Sk, Dh = 32, 8, 65536, 128
        assert Hq % Hkv == 0, (Hq, Hkv)
        return {
            "x": _w((lambda *s: _rng.normal(s) * 0.05)(B, Sq, D)),
            "k_cache": _w((lambda *s: _rng.normal(s) * 1.6)(B, Hkv, Sk, Dh)),
            "v_cache": _w((lambda *s: _rng.normal(s) * 1.6)(B, Hkv, Sk, Dh)),
            "wq": _w((lambda *s: _rng.normal(s) * 1.6)(D, Hq * Dh) * (D ** -0.5)),
            "wo": _w((lambda *s: _rng.normal(s) * 1.6)(Hq * Dh, D) * ((Hq * Dh) ** -0.5)),
        }
    _A_in = _A_setup()

    def _B_setup():
        B, S, D, F = 1, 1, 512, 1792
        return {
            "x": _w((lambda *s: _rng.normal(s) * 0.05)(B, S, D)),
            "w1": _w((lambda *s: _rng.normal(s) * 0.8)(D, F) * (D ** -0.5)),
            "b1": _w((lambda *s: _rng.normal(s) * 0.8)(F)),
            "w2": _w((lambda *s: _rng.normal(s) * 0.8)(F, D) * (F ** -0.5)),
        }
    _B_in = _B_setup()

    return {
        "A_x": _A_in["x"],
        "A_k_cache": _A_in["k_cache"],
        "A_v_cache": _A_in["v_cache"],
        "A_wq": _A_in["wq"],
        "A_wo": _A_in["wo"],
        "B_x": _B_in["x"],
        "B_w1": _B_in["w1"],
        "B_b1": _B_in["b1"],
        "B_w2": _B_in["w2"],
    }

def reference(A_x, A_k_cache, A_v_cache, A_wq, A_wo, B_x, B_w1, B_b1, B_w2):
    def _A_ref(x, k_cache, v_cache, wq, wo):
        B, Sq, D = x.shape
        Hq, Dh = 32, 128
        Hkv = k_cache.shape[1]
        rep = Hq // Hkv
        q = (lambda x, *d: x.transpose(*d))((x @ wq).reshape(B, Sq, Hq, Dh), 0, 2, 1, 3)
        k = jnp.repeat(k_cache, rep, axis=1)
        v = jnp.repeat(v_cache, rep, axis=1)
        scores = jnp.einsum("bhqd,bhkd->bhqk", q, k) * (Dh ** -0.5)
        p = _softmax(scores, axis=-1)
        o = jnp.einsum("bhqk,bhkd->bhqd", p, v)
        return (lambda x, *d: x.transpose(*d))(o, 0, 2, 1, 3).reshape(B, Sq, Hq * Dh) @ wo

    def _B_ref(x, w1, b1, w2):
        h = jnp.einsum("bsd,df->bsf", x, w1) + b1
        sp = jnp.log1p(jnp.exp(-jnp.abs(h))) + jnp.where(h > 0, h, jnp.zeros_like(h))
        act = h * jnp.tanh(sp)
        return jnp.einsum("bsf,fd->bsd", act, w2)

    x = A_x
    x = x + _A_ref(_layernorm(x, axis=-1), A_k_cache, A_v_cache, A_wq, A_wo)
    x = x + _B_ref(_layernorm(x, axis=-1), B_w1, B_b1, B_w2)
    x = x + _A_ref(_layernorm(x, axis=-1), A_k_cache, A_v_cache, A_wq, A_wo)
    x = x + _B_ref(_layernorm(x, axis=-1), B_w1, B_b1, B_w2)
    return x
```

```python
import functools

import jax
import jax.numpy as jnp
from jax import lax
import jax.experimental.pallas as pl
import jax.experimental.pallas.tpu as pltpu


_T = 2048
_SLOTS = 116
_AHEAD = 4
_RING = 4
_NSEM = 8
_TRANS_B = (((1,), (1,)), ((), ()))


def _layernorm(x):
    m = jnp.mean(x, axis=-1, keepdims=True)
    d = x - m
    v = jnp.mean(d * d, axis=-1, keepdims=True)
    return d / jnp.sqrt(v + 1e-5)


def _kernel(x_ref, b1_ref, k_hbm, v_hbm, wq_hbm, wo_hbm, w1_hbm, w2_hbm,
            o_ref,
            kbuf, vbuf, wq_v, wo_v, w1_v, w2_v,
            q_scr, m_scr, l_scr, acc_scr, kv_sem, w_sem,
            *, T, n_slots, ahead, ring):
    _, hkv, sk, dh = k_hbm.shape
    d_model = x_ref.shape[-1]
    hq = wq_hbm.shape[1] // dh
    rep = hq // hkv
    cph = sk // T
    nch = hkv * cph
    n_str = nch - n_slots
    scale = dh ** -0.5
    f32, bf16 = jnp.float32, jnp.bfloat16

    def kv_copies(chunk, slot, sem):
        g = chunk // cph
        r0 = pl.multiple_of((chunk % cph) * T, T)
        return (
            pltpu.make_async_copy(k_hbm.at[0, g, pl.ds(r0, T), :], kbuf.at[slot],
                                  kv_sem.at[0, sem]),
            pltpu.make_async_copy(v_hbm.at[0, g, pl.ds(r0, T), :], vbuf.at[slot],
                                  kv_sem.at[1, sem]),
        )

    def start_kv(chunk, slot, sem):
        for c in kv_copies(chunk, slot, sem):
            c.start()

    def wait_kv(chunk, slot, sem):
        for c in kv_copies(chunk, slot, sem):
            c.wait()

    w_copies = [
        pltpu.make_async_copy(wq_hbm, wq_v, w_sem.at[0]),
        pltpu.make_async_copy(wo_hbm, wo_v, w_sem.at[1]),
        pltpu.make_async_copy(w1_hbm, w1_v, w_sem.at[2]),
        pltpu.make_async_copy(w2_hbm, w2_v, w_sem.at[3]),
    ]

    def setup_attention(x):
        xn = _layernorm(x).astype(bf16)
        q_all = jnp.dot(xn, wq_v[...], preferred_element_type=f32)
        row = lax.broadcasted_iota(jnp.int32, (8, dh), 0)
        for g in range(hkv):
            qg = jnp.zeros((8, dh), f32)
            for r in range(rep):
                h = g * rep + r
                qg = jnp.where(row == r, q_all[:, h * dh:(h + 1) * dh], qg)
            q_scr[g] = qg
        m_scr[...] = jnp.full(m_scr.shape, -jnp.inf, f32)
        l_scr[...] = jnp.zeros(l_scr.shape, f32)
        acc_scr[...] = jnp.zeros(acc_scr.shape, f32)

    def process(slot, g):
        q = q_scr[g].astype(bf16)
        k = kbuf[slot]
        s = lax.dot_general(q, k, _TRANS_B, preferred_element_type=f32) * scale
        m_old = m_scr[g]
        m_new = jnp.maximum(m_old, jnp.max(s, axis=-1, keepdims=True))
        alpha = jnp.exp(m_old - m_new)
        p = jnp.exp(s - m_new[:, 0:1])
        l_scr[g] = alpha * l_scr[g] + jnp.sum(p, axis=-1, keepdims=True)
        pv = jnp.dot(p.astype(bf16), vbuf[slot], preferred_element_type=f32)
        acc_scr[g] = alpha * acc_scr[g] + pv
        m_scr[g] = m_new

    def finish_attention_and_ffn(x):
        parts = []
        for g in range(hkv):
            og = acc_scr[g] / l_scr[g]
            for r in range(rep):
                parts.append(jnp.broadcast_to(og[r:r + 1, :], (8, dh)))
        o_flat = jnp.concatenate(parts, axis=1).astype(bf16)
        x = x + jnp.dot(o_flat, wo_v[...], preferred_element_type=f32)
        xn = _layernorm(x).astype(bf16)
        h = jnp.dot(xn, w1_v[...], preferred_element_type=f32)
        h = h + b1_ref[...].astype(f32)
        sp = jnp.log1p(jnp.exp(-jnp.abs(h))) + jnp.where(h > 0, h, 0.0)
        act = (h * jnp.tanh(sp)).astype(bf16)
        return x + jnp.dot(act, w2_v[...], preferred_element_type=f32)

    w_copies[0].start()
    for c in range(ahead):
        start_kv(c, c, c)
    for c in w_copies[1:]:
        c.start()
    x = jnp.broadcast_to(x_ref[0].astype(f32), (8, d_model))
    w_copies[0].wait()

    setup_attention(x)

    def pass1(c, carry):
        @pl.when(c + ahead < nch)
        def _():
            cn = c + ahead
            start_kv(cn, cn % n_slots, cn % _NSEM)
        wait_kv(c, c % n_slots, c % _NSEM)
        process(c % n_slots, c // cph)
        return carry

    lax.fori_loop(0, nch, pass1, 0)

    for c in w_copies[1:]:
        c.wait()
    x = finish_attention_and_ffn(x)

    setup_attention(x)

    def cached(i):
        c = n_str + i
        return c % n_slots, c // cph

    def ring_slot(s):
        return (n_str + s % ring) % n_slots

    for i in range(ring):
        process(*cached(i))
        if i < n_str:
            start_kv(i, ring_slot(i), i % _NSEM)

    n_rest = n_slots - ring
    n_spread = max(n_str - 2, 1)

    def pass2(s, carry):
        wait_kv(s, ring_slot(s), s % _NSEM)
        process(ring_slot(s), s // cph)

        @pl.when(s + ring < n_str)
        def _():
            start_kv(s + ring, ring_slot(s), (s + ring) % _NSEM)

        lo = jnp.minimum((s * n_rest) // n_spread, n_rest)
        hi = jnp.minimum(((s + 1) * n_rest) // n_spread, n_rest)

        def inner(i, c2):
            process(*cached(ring + i))
            return c2
        lax.fori_loop(lo, hi, inner, 0)
        return carry

    lax.fori_loop(0, n_str, pass2, 0)

    x = finish_attention_and_ffn(x)
    o_ref[0] = x[0:1, :].astype(o_ref.dtype)


def _build(x, k, v, wq, wo, w1, b1, w2, *, T=_T, n_slots=_SLOTS, ahead=_AHEAD,
           ring=_RING):
    dh = k.shape[-1]
    hkv = k.shape[1]
    any_spec = pl.BlockSpec(memory_space=pl.ANY)
    vmem_spec = pl.BlockSpec(memory_space=pltpu.VMEM)
    return pl.pallas_call(
        functools.partial(_kernel, T=T, n_slots=n_slots, ahead=ahead, ring=ring),
        out_shape=jax.ShapeDtypeStruct(x.shape, x.dtype),
        in_specs=[vmem_spec, vmem_spec] + [any_spec] * 6,
        out_specs=vmem_spec,
        scratch_shapes=[
            pltpu.VMEM((n_slots, T, dh), k.dtype),
            pltpu.VMEM((n_slots, T, dh), v.dtype),
            pltpu.VMEM(wq.shape, wq.dtype),
            pltpu.VMEM(wo.shape, wo.dtype),
            pltpu.VMEM(w1.shape, w1.dtype),
            pltpu.VMEM(w2.shape, w2.dtype),
            pltpu.VMEM((hkv, 8, dh), jnp.float32),
            pltpu.VMEM((hkv, 8, dh), jnp.float32),
            pltpu.VMEM((hkv, 8, dh), jnp.float32),
            pltpu.VMEM((hkv, 8, dh), jnp.float32),
            pltpu.SemaphoreType.DMA((2, _NSEM)),
            pltpu.SemaphoreType.DMA((4,)),
        ],
        compiler_params=pltpu.CompilerParams(
            vmem_limit_bytes=128 * 1024 * 1024,
        ),
    )(x, b1.reshape(1, -1), k, v, wq, wo, w1, w2)


@jax.jit
def pallas_interleave_layers__gqa_block_cached__dense_activation_mish__decode_kernel(
    A_x: jax.Array,
    A_k_cache: jax.Array,
    A_v_cache: jax.Array,
    A_wq: jax.Array,
    A_wo: jax.Array,
    B_x: jax.Array,
    B_w1: jax.Array,
    B_b1: jax.Array,
    B_w2: jax.Array,
):
    del B_x
    return _build(A_x, A_k_cache, A_v_cache, A_wq, A_wo, B_w1, B_b1, B_w2)
```

```python
import functools

import jax
import jax.numpy as jnp
from jax import lax
import jax.experimental.pallas as pl
import jax.experimental.pallas.tpu as pltpu


_T = 2048
_NCOMP = 164
_RING = 3
_HEAD = 1
_EARLY = True
_LATE = 14
_REST_POS = 2
_TRANS_B = (((1,), (1,)), ((), ()))
_U32 = jnp.uint32


def _layernorm(x):
    m = jnp.mean(x, axis=-1, keepdims=True)
    d = x - m
    v = jnp.mean(d * d, axis=-1, keepdims=True)
    return d / jnp.sqrt(v + 1e-5)


_H = 0x00010001


def _c(x):
    return _U32((x * _H) & 0xFFFFFFFF)


def _pack_group(w, kv, st):
    exc, low, high, cnt = st
    ts = [None] * 16
    for j in reversed(range(16)):
        u = (w[j] & _c(0x7FFF)) + kv
        low = low | (u - _c(16 << 7))
        high = high | (u + _c(17 << 7))
        m = (u & _c(0x1000)) ^ _c(0x1000)
        m5 = m >> _U32(5)
        ts[j] = ((u | ((m >> _U32(1)) - m5)) & _c(0x07FF)) | (w[j] & _c(0x8000))
        rec = u & (m - m5)
        cnt = cnt + m5
        exc = jnp.where(m != 0, (exc << _U32(5)) | (rec >> _U32(7)), exc)
    out = []
    for s in range(4):
        t = ts[12 + s]
        v = (t & _c(0x07FF)) | ((t >> _U32(4)) & _c(0x0800))
        for k, sh in enumerate((11, 7, 3)):
            out.append(ts[3 * s + k] | ((v << _U32(sh)) & _c(0x7800)))
    return out, (exc, low, high, cnt)


def _pack_bad(st):
    _, low, high, cnt = st
    n = ((cnt >> _U32(7)) & _U32(0x1FF)) + (cnt >> _U32(23))
    bad = (low & _c(0xF000)) | (high & _c(0xE000)) | ((_U32(3) - n) & _U32(0x8000))
    return (bad | (bad >> _U32(16))) & _U32(0xFFFF)


def _open_queue(exc, basev):
    bs = []
    for sh in (7, 2, -3):
        r = (exc << _U32(sh) if sh > 0 else exc >> _U32(-sh)) & _c(0x0F80)
        e = r & _c(0x0800)
        bs.append(basev + r + (e >> _U32(4)) - e - (e << _U32(1)))
    return tuple(bs)


def _unpack_group(c, bs, basev):
    ts = [x & _c(0x87FF) for x in c]
    for s in range(4):
        ts.append(((c[3 * s] & _c(0x7800)) >> _U32(11))
                  | ((c[3 * s + 1] & _c(0x7800)) >> _U32(7))
                  | ((c[3 * s + 2] & _c(0x3800)) >> _U32(3))
                  | ((c[3 * s + 2] & _c(0x4000)) << _U32(1)))
    out = []
    b0, b1, b2 = bs
    for t in ts:
        y = t + _c(0x0080)
        hit = (y & _c(0x0800)) != 0
        out.append(y + jnp.where(hit, b0, basev))
        b0, b1 = jnp.where(hit, b1, b0), jnp.where(hit, b2, b1)
    return out, (b0, b1, b2)


def _kernel(x_ref, b1_ref, k_hbm, v_hbm, wq_hbm, wo_hbm, w1_hbm, w2_hbm,
            o_ref,
            kbuf, vbuf, kpack, vpack,
            q_scr, m_scr, l_scr, acc_scr, meta, lists, sem,
            *, T, n_comp, ring):
    _, hkv, sk, dh = k_hbm.shape
    d_model = x_ref.shape[-1]
    d_ff = w1_hbm.shape[1]
    hq = wq_hbm.shape[1] // dh
    rep = hq // hkv
    cph = sk // T
    nch = hkv * cph
    n_str = nch - n_comp
    n_grp = T // 256
    scale2 = dh ** -0.5 * 1.4426950408889634
    f32, bf16 = jnp.float32, jnp.bfloat16
    bufs = (kbuf, vbuf)
    bufs_u32 = tuple(b.bitcast(_U32) for b in bufs)

    def col_blocks(w_hbm, r0, nr):
        return [(r0, nr, j) for j in range(w_hbm.shape[1] // dh)]

    def cut(blocks):
        pieces, cur, half, used = [], [], 0, 0
        for (r0, nr, j) in blocks:
            if used + nr > T:
                half, used = half + 1, 0
                if half == 2:
                    pieces.append(cur)
                    cur, half = [], 0
            cur.append((half, used, r0, nr, j))
            used += nr
        pieces.append(cur)
        return pieces

    wq_pieces = cut(col_blocks(wq_hbm, 0, d_model))
    wo_rows = 2 * T * dh // d_model
    wo_pieces = [p for r0 in range(0, hq * dh, wo_rows)
                 for p in cut(col_blocks(wo_hbm, r0, wo_rows))]
    w1_pieces = cut(col_blocks(w1_hbm, 0, d_model))
    w2_pieces = cut(col_blocks(w2_hbm, 0, d_ff))
    post = ([(wo_hbm, p) for p in wo_pieces] + [(w1_hbm, p) for p in w1_pieces]
            + [(w2_hbm, p) for p in w2_pieces])
    pre = [(wq_hbm, p) for p in wq_pieces[::-1]]
    assert ring <= len(pre) and ring <= len(post)
    assert all(len(p) == T // d_model * 2 for p in wq_pieces)

    def w_copies(piece, slot, only=None):
        w_hbm, blocks = piece
        blocks = [b for b in blocks if only is None or b[0] == only]
        return [pltpu.make_async_copy(
                    w_hbm.at[pl.ds(r0, nr), pl.ds(j * dh, dh)],
                    bufs[half].at[slot, pl.ds(dst, nr), :], sem.at[half, slot])
                for (half, dst, r0, nr, j) in blocks]

    def kv_copy(half, chunk, slot):
        g = chunk // cph
        r0 = pl.multiple_of((chunk % cph) * T, T)
        return pltpu.make_async_copy((k_hbm, v_hbm)[half].at[0, g, pl.ds(r0, T), :],
                                     bufs[half].at[slot], sem.at[half, slot])

    def kv_copies(chunk, slot):
        return [kv_copy(0, chunk, slot), kv_copy(1, chunk, slot)]

    def start(copies):
        for c in copies:
            c.start()

    def wait(copies):
        for c in copies:
            c.wait()

    def w_block(piece, slot, blk):
        half, dst, _, nr, _ = blk
        return pltpu.bitcast(bufs_u32[half][slot, pl.ds(dst // 2, nr // 2), :], bf16)

    def project_q(x, first, issue, between=None):
        xn = _layernorm(x).astype(bf16)
        row = lax.broadcasted_iota(jnp.int32, (8, dh), 0)
        m_scr[...] = jnp.full(m_scr.shape, -jnp.inf, f32)
        l_scr[...] = jnp.zeros(l_scr.shape, f32)
        acc_scr[...] = jnp.zeros(acc_scr.shape, f32)
        for i, piece in enumerate(pre):
            slot = (first + i) % ring
            wait(w_copies(piece, slot))
            qs = {}
            for blk in piece[1]:
                g, r = divmod(blk[4], rep)
                qr = jnp.dot(xn, w_block(piece, slot, blk), preferred_element_type=f32)
                qs[g] = jnp.where(row == r, qr, qs.get(g, jnp.zeros((8, dh), f32)))
            issue(i + ring, slot)
            for g, qg in qs.items():
                q_scr[g] = qg
            if between is not None:
                between(i)

    def out_proj_and_ffn(x, first, issue, live, between=None):
        def o_cols(r0, nr):
            parts = []
            for g in range(r0 // (rep * dh), (r0 + nr) // (rep * dh)):
                og = acc_scr[g] / l_scr[g]
                parts += [jnp.broadcast_to(og[r:r + 1, :], (8, dh)) for r in range(rep)]
            return jnp.concatenate(parts, axis=1).astype(bf16)
        nblk = d_model // dh
        pos = 0

        def matmul_pieces(pieces, lhs_fn, n_out):
            nonlocal pos
            outs = [None] * n_out
            for piece in pieces:
                slot = (first + pos) % ring
                if between is not None:
                    between(pos)
                wait(w_copies(piece, slot))
                lhs = {blk[2:4]: lhs_fn(*blk[2:4]) for blk in piece[1]}

                def dots():
                    return [jnp.dot(lhs[blk[2:4]], w_block(piece, slot, blk),
                                    preferred_element_type=f32) for blk in piece[1]]
                ys = lax.cond(live, dots,
                              lambda: [jnp.zeros((8, dh), f32)] * len(piece[1]))
                for blk, y in zip(piece[1], ys):
                    j = blk[4]
                    outs[j] = y if outs[j] is None else outs[j] + y
                issue(pos + ring, slot)
                pos += 1
            return jnp.concatenate(outs, axis=1)

        n_wo, n_w1 = len(wo_pieces), len(w1_pieces)
        x = x + matmul_pieces(
            post[:n_wo],
            o_cols,
            nblk)
        xn = _layernorm(x).astype(bf16)
        h = matmul_pieces(post[n_wo:n_wo + n_w1], lambda r0, nr: xn, d_ff // dh)
        h = h + b1_ref[...].astype(f32).reshape(1, -1)
        sp = jnp.log1p(jnp.exp(-jnp.abs(h))) + jnp.where(h > 0, h, 0.0)
        act = (h * jnp.tanh(sp)).astype(bf16)
        return x + matmul_pieces(post[n_wo + n_w1:], lambda r0, nr: act, nblk)

    def attend(*chunks):
        ss = []
        for k_fn, _, g in chunks:
            q = q_scr[g].astype(bf16)
            ss.append([lax.dot_general(q, k_fn(b), _TRANS_B, preferred_element_type=f32)
                       * scale2 for b in range(n_grp)])
        for s_grp, (_, v_fn, g) in zip(ss, chunks):
            m_old = m_scr[g]
            mx = functools.reduce(jnp.maximum, s_grp)
            m_new = jnp.maximum(m_old, jnp.max(mx, axis=-1, keepdims=True))
            alpha = jnp.exp2(m_old - m_new)
            ps = [jnp.exp2(s - m_new[:, 0:1]) for s in s_grp]
            l_scr[g] = alpha * l_scr[g] + jnp.sum(
                functools.reduce(jnp.add, ps), axis=-1, keepdims=True)
            pv = functools.reduce(jnp.add, [
                jnp.dot(p.astype(bf16), v_fn(b), preferred_element_type=f32)
                for b, p in enumerate(ps)])
            acc_scr[g] = alpha * acc_scr[g] + pv
            m_scr[g] = m_new

    def splat2(x):
        return jnp.full((8, dh), x * (128 * _H), jnp.int32).astype(_U32)

    def pick_base(half, slot, g):
        w0 = bufs_u32[half][slot, pl.ds(0, 8), :]
        e = jnp.maximum(((w0 >> _U32(23)) & _U32(0xFF)).astype(jnp.int32),
                        ((w0 >> _U32(7)) & _U32(0xFF)).astype(jnp.int32))
        top = jnp.max(e.astype(f32)).astype(jnp.int32)
        meta[half, g] = jnp.clip(top + (_HEAD - 14), 0, 241)

    def pack_chunk(half, slot, i, g):
        src, dst = bufs_u32[half], (kpack, vpack)[half]
        kv = splat2(32 - meta[half, g])
        st = (jnp.zeros((8, dh), _U32),) * 4
        for b in reversed(range(n_grp)):
            w = [src[slot, pl.ds(b * 128 + j * 8, 8), :] for j in range(16)]
            out, st = _pack_group(w, kv, st)
            for j in range(12):
                dst[i, pl.ds(b * 96 + j * 8, 8), :] = out[j]
        dst[i, pl.ds(n_grp * 96, 8), :] = st[0]
        return _pack_bad(st)

    def unpack_fn(src, i, base):
        state = {}

        def group(b):
            if b == 0:
                state["basev"] = splat2(base - 1)
                state["bs"] = _open_queue(src[i, pl.ds(n_grp * 96, 8), :], state["basev"])
            c = [src[i, pl.ds(b * 96 + j * 8, 8), :] for j in range(12)]
            out, state["bs"] = _unpack_group(c, state["bs"], state["basev"])
            return jnp.concatenate([pltpu.bitcast(w, bf16) for w in out], axis=0)
        return group

    def raw(slot, c):
        def load(half, b):
            return pltpu.bitcast(bufs_u32[half][slot, pl.ds(b * 128, 128), :], bf16)
        return functools.partial(load, 0), functools.partial(load, 1), c // cph

    def packed(n):
        i, g = lists[1, n], lists[2, n]
        return unpack_fn(kpack, i, meta[0, g]), unpack_fn(vpack, i, meta[1, g]), g

    for i in range(ring):
        start(w_copies(pre[i], i))

    def init_lists(i, carry):
        for r in range(3):
            lists[r, i] = 0
        return carry
    lax.fori_loop(0, nch, init_lists, 0)
    x = jnp.broadcast_to(x_ref[0].astype(f32), (8, d_model))

    n_pre, n_post = len(pre), len(post)

    def issue_pre1(i, slot):
        if i < n_pre:
            start(w_copies(pre[i], slot))
        else:
            start(kv_copies(i - n_pre, slot))
    project_q(x, 0, issue_pre1)

    def release(slot, nxt, chunk_fn, n_kv):
        @pl.when(nxt < n_kv)
        def _():
            start(kv_copies(chunk_fn(nxt), slot))

        def weights(_, carry):
            lax.switch(jnp.clip(nxt - n_kv, 0, ring - 1),
                       [functools.partial(start, w_copies(post[i], slot))
                        for i in range(ring)])
            return carry
        lax.fori_loop(0, (nxt >= n_kv).astype(jnp.int32), weights, 0)

    def pass1(c, counts):
        slot = (n_pre + c) % ring
        g = c // cph
        i = (c * n_comp) // nch
        chosen = ((c + 1) * n_comp) // nch > i

        kv_copy(0, c, slot).wait()
        kv_copy(1, c, slot).wait()

        @pl.when(c % cph == 0)
        def _():
            pick_base(0, slot, g)
            pick_base(1, slot, g)

        def with_pack():
            chk = pack_chunk(0, slot, i, g) | pack_chunk(1, slot, i, g)
            attend(raw(slot, c))
            return jnp.max(chk.astype(jnp.int32).astype(f32))

        def plain():
            attend(raw(slot, c))
            return jnp.float32(0)
        bad = lax.cond(chosen, with_pack, plain) > 0
        release(slot, c + ring, lambda n: n, nch)

        n_stream, n_ok = counts
        lists[0, n_stream] = c
        lists[1, jnp.minimum(n_ok, n_comp - 1)] = i
        lists[2, jnp.minimum(n_ok, n_comp - 1)] = g
        ok = jnp.logical_and(chosen, jnp.logical_not(bad)).astype(jnp.int32)
        return n_stream + 1 - ok, n_ok + ok

    n_stream, n_ok = lax.fori_loop(0, nch, pass1, (jnp.int32(0), jnp.int32(0)))

    def stream_chunk(s):
        return lists[0, s]

    pos_post1 = n_pre + nch
    pos_pre2 = pos_post1 + n_post
    pos_str = pos_pre2 + n_pre

    def issue_post1(i, slot):
        start(w_copies(post[i] if i < n_post else pre[i - n_post], slot))
    x = out_proj_and_ffn(x, pos_post1, issue_post1, n_ok >= 0)

    def issue_pre2(i, slot):
        if i < n_pre:
            start(w_copies(pre[i], slot))
        else:
            start(kv_copies(stream_chunk(i - n_pre), slot))
    early = {"n": n_ok}

    def early_pairs(i):
        n = early["n"]
        g_min = hkv - (i + 1) * (hkv // n_pre)
        ok = jnp.logical_and(
            n >= 2, lists[2, jnp.maximum(n - 2, 0)] >= g_min)

        def pair():
            attend(packed(n - 1), packed(n - 2))
            return n - 2
        early["n"] = lax.cond(ok, pair, lambda: n)
    project_q(x, pos_pre2, issue_pre2, early_pairs if _EARLY else None)
    n_ok = early["n"]


    def pass2(s, done):
        slot = (pos_str + s) % ring
        c = stream_chunk(s)
        wait(kv_copies(c, slot))

        def both():
            attend(raw(slot, c), packed(done))
            return done + 1

        def only_raw():
            attend(raw(slot, c))
            return done
        done = lax.cond(done < n_ok, both, only_raw)
        release(slot, s + ring, stream_chunk, n_stream)

        target = jnp.minimum(((s + 1) * (n_comp - _LATE)) // n_str, n_ok)

        def more(done):
            return done + 2 <= target

        def extra(done):
            attend(packed(done), packed(done + 1))
            return done + 2
        return lax.while_loop(more, extra, done)

    done = lax.fori_loop(0, n_stream, pass2, jnp.int32(0))

    left = {"done": done}

    def rest(pos):
        if pos not in (0, _REST_POS):
            return
        done = left["done"]
        stop = n_ok
        if pos == 0:
            g_need = _REST_POS * wo_rows // (rep * dh)
            stop = jnp.where(lists[2, jnp.minimum(done, nch - 1)] < g_need, n_ok, done)

        def two(i, carry):
            attend(packed(done + 2 * i), packed(done + 2 * i + 1))
            return carry
        lax.fori_loop(0, (stop - done) // 2, two, 0)

        @pl.when((stop - done) % 2 == 1)
        def _():
            attend(packed(jnp.maximum(stop - 1, 0)))
        left["done"] = stop

    def issue_post2(i, slot):
        if i < n_post:
            start(w_copies(post[i], slot))
    x = out_proj_and_ffn(x, pos_str + n_stream, issue_post2, n_ok >= 0, rest)
    o_ref[0] = x[0:1, :].astype(o_ref.dtype)


def _build(x, k, v, wq, wo, w1, b1, w2, *, T=_T, n_comp=_NCOMP, ring=_RING):
    dh = k.shape[-1]
    hkv = k.shape[1]
    nch = hkv * (k.shape[2] // T)
    assert nch - n_comp >= ring
    any_spec = pl.BlockSpec(memory_space=pl.ANY)
    vmem_spec = pl.BlockSpec(memory_space=pltpu.VMEM)
    return pl.pallas_call(
        functools.partial(_kernel, T=T, n_comp=n_comp, ring=ring),
        out_shape=jax.ShapeDtypeStruct(x.shape, x.dtype),
        in_specs=[vmem_spec, vmem_spec] + [any_spec] * 6,
        out_specs=vmem_spec,
        scratch_shapes=[
            pltpu.VMEM((ring, T, dh), k.dtype),
            pltpu.VMEM((ring, T, dh), v.dtype),
            pltpu.VMEM((n_comp, 12 * T // 32 + 8, dh), _U32),
            pltpu.VMEM((n_comp, 12 * T // 32 + 8, dh), _U32),
            pltpu.VMEM((hkv, 8, dh), jnp.float32),
            pltpu.VMEM((hkv, 8, dh), jnp.float32),
            pltpu.VMEM((hkv, 8, dh), jnp.float32),
            pltpu.VMEM((hkv, 8, dh), jnp.float32),
            pltpu.SMEM((2, hkv), jnp.int32),
            pltpu.SMEM((3, nch), jnp.int32),
            pltpu.SemaphoreType.DMA((2, ring)),
        ],
        compiler_params=pltpu.CompilerParams(
            vmem_limit_bytes=128 * 1024 * 1024,
            flags={"XLA_TPU_FORCE_LP_LLO_SCHEDULER": True},
        ),
    )(x, b1, k, v, wq, wo, w1, w2)


@jax.jit
def pallas_interleave_layers__gqa_block_cached__dense_activation_mish__decode_kernel(
    A_x: jax.Array,
    A_k_cache: jax.Array,
    A_v_cache: jax.Array,
    A_wq: jax.Array,
    A_wo: jax.Array,
    B_x: jax.Array,
    B_w1: jax.Array,
    B_b1: jax.Array,
    B_w2: jax.Array,
):
    del B_x
    return _build(A_x, A_k_cache, A_v_cache, A_wq, A_wo, B_w1, B_b1, B_w2)
```
